```python
import os as _os
_os.environ.setdefault("JAX_PLATFORMS", "cpu")
import jax
import jax.numpy as jnp

def _softmax(x, axis=-1):
    return jax.nn.softmax(x, axis=axis)
def _gelu(x):
    return jax.nn.gelu(x, approximate=True)
def _silu(x):
    return jax.nn.silu(x)
def _sigmoid(x):
    return jax.nn.sigmoid(x)
def _layernorm(x, axis=-1, eps=1e-5):
    m = jnp.mean(x, axis=axis, keepdims=True)
    v = jnp.var(x, axis=axis, keepdims=True)
    return (x - m) / jnp.sqrt(v + eps)
def _scatter_add(tgt, idx, src, axis=0):
    return tgt.at[idx].add(src)
def _segment_sum(src, seg, n):
    return jax.ops.segment_sum(src, seg, n)
class _Rng:
    def __init__(self, key):
        self._k = key
    def _next(self):
        self._k, sub = jax.random.split(self._k)
        return sub
    def normal(self, shape):
        return jax.random.normal(self._next(), shape, dtype=jnp.bfloat16)
    def randint(self, lo, hi, shape):
        return jax.random.randint(self._next(), shape, lo, hi, dtype=jnp.int32)
    def uniform(self, shape, lo=0.0, hi=1.0):
        return jax.random.uniform(self._next(), shape, jnp.bfloat16, lo, hi)
    def permutation(self, n):
        return jax.random.permutation(self._next(), n)


kernel_name = 'sequential_preLN__mha_block__moe_arch_mod__prompt'

def setup_inputs():
    _rng = _Rng(jax.random.key(int.from_bytes(__import__("os").urandom(4), "little")))
    _w = (lambda a: (lambda t: t.astype(jnp.bfloat16) if jnp.issubdtype(t.dtype, jnp.floating) else t)(jnp.asarray(a)))
    def _A_setup():
        B, S, D, H = 1, 2048, 640, 32
        return {
            "x": _w((lambda *s: _rng.normal(s) * 0.05)(B, S, D)),
            "wqkv": _w((lambda *s: _rng.normal(s) * 0.05)(D, 3 * D)),
            "wo": _w((lambda *s: _rng.normal(s) * 0.05)(D, D)),
        }
    _A_in = _A_setup()

    def _B_setup():
        B, S, D, F, C = 1, 2048, 640, 1536, 1
        return {
            "x": _w((lambda *s: _rng.normal(s) * 0.05)(B, S, D)),
            "w_r": _w((lambda *s: _rng.normal(s) * 0.05)(D)),
            "w_gate": _w((lambda *s: _rng.normal(s) * 0.05)(D, F)),
            "w_up": _w((lambda *s: _rng.normal(s) * 0.05)(D, F)),
            "w_down": _w((lambda *s: _rng.normal(s) * 0.05)(F, D)),
        }
    _B_in = _B_setup()

    return {
        "A_x": _A_in["x"],
        "A_wqkv": _A_in["wqkv"],
        "A_wo": _A_in["wo"],
        "B_x": _B_in["x"],
        "B_w_r": _B_in["w_r"],
        "B_w_gate": _B_in["w_gate"],
        "B_w_up": _B_in["w_up"],
        "B_w_down": _B_in["w_down"],
    }

def reference(A_x, A_wqkv, A_wo, B_x, B_w_r, B_w_gate, B_w_up, B_w_down):
    def _A_ref(x, wqkv, wo):
        B, S, D = x.shape
        H = 32
        Dh = D // H
        qkv = (lambda x, *d: x.transpose(*d))((x @ wqkv).reshape(B, S, 3, H, Dh), 2, 0, 3, 1, 4)
        q, k, v = qkv[0], qkv[1], qkv[2]
        scores = jnp.einsum("bhqd,bhkd->bhqk", q, k) * (Dh ** -0.5)
        p = _softmax(scores, axis=-1)
        o = jnp.einsum("bhqk,bhkd->bhqd", p, v)
        return (lambda x, *d: x.transpose(*d))(o, 0, 2, 1, 3).reshape(B, S, D) @ wo

    def _B_ref(x, w_r, w_gate, w_up, w_down):
        B, S, D = x.shape
        C = 1
        r = x @ w_r
        idx = jnp.argsort(-r, axis=-1)[:, :C]
        idx_e = jnp.repeat(idx.reshape(B, C, 1), D, axis=2)
        x_sel = jnp.take_along_axis(x, idx_e, axis=1)
        g = _silu(x_sel @ w_gate)
        u = x_sel @ w_up
        y = (g * u) @ w_down
        r_sel = _sigmoid(jnp.take_along_axis(r, idx, axis=1))
        y = y * r_sel.reshape(B, C, 1)
        b_off = (jnp.arange(B) * S).reshape(B, 1)
        flat_idx = (idx + b_off).reshape(B * C)
        zero = (x * 0.0).reshape(B * S, D)
        upd = _scatter_add(zero, flat_idx, y.reshape(B * C, D), axis=0)
        return x + upd.reshape(B, S, D)

    x = A_x
    h = x + _A_ref(_layernorm(x, axis=-1), A_wqkv, A_wo)
    h2 = h + _B_ref(_layernorm(h, axis=-1), B_w_r, B_w_gate, B_w_up, B_w_down)
    return h2
```

```python
import jax
import jax.numpy as jnp
import numpy as np
from jax import lax
from jax.experimental import pallas as pl
from jax.experimental.pallas import tpu as pltpu

S, D, H, DH, F = 2048, 640, 32, 20, 1536
EPS = 1e-5
LANES = 128

RB = 256
NRB = S // RB
KC = 128
QG = 256
NQG = S // QG
NWIN = 9
VW = 24
Q_SCALE = float(DH ** -0.5 * np.log2(np.e))

ROUTE_AT = 2
BF16, F32, U32, I32 = jnp.bfloat16, jnp.float32, jnp.uint32, jnp.int32


def _layernorm(x):
    mu = jnp.mean(x, axis=-1, keepdims=True)
    xc = x - mu
    var = jnp.mean(xc * xc, axis=-1, keepdims=True)
    return xc * lax.rsqrt(var + EPS)


def _pack(x):
    return pltpu.bitcast(x.astype(BF16), U32)


def _unpack(x):
    return pltpu.bitcast(x, BF16)


def _kernel(x_hbm, wqkv_hbm, wo_hbm, wr_hbm, wg_hbm, wu_hbm, wd_hbm, out_hbm,
            x_v, w_v, wo_v, wr_v, wg_v, wu_v, wd_v,
            xn_v, kwin, qt, vt, ot, s_v, m_v, wot_v, at_v, hn_v, r_v, o_v, fix_v,
            sem_x, sem_w, sem_o, sem_fix):

    def x_copy(b):
        rows = pl.ds(pl.multiple_of(b * RB, RB), RB)
        return pltpu.make_async_copy(x_hbm.at[rows], x_v.at[rows], sem_x.at[b])

    def out_copy(g):
        rows = pl.ds(pl.multiple_of(g * QG, QG), QG)
        return pltpu.make_async_copy(o_v.at[rows], out_hbm.at[rows], sem_o.at[g])

    def wqkv_copy(j):
        return pltpu.make_async_copy(wqkv_hbm.at[:, pl.ds(j * D, D)], w_v.at[j], sem_w.at[j])

    late_copies = [
        pltpu.make_async_copy(wo_hbm, wo_v, sem_w.at[3]),
        pltpu.make_async_copy(wr_hbm, wr_v, sem_w.at[4]),
        pltpu.make_async_copy(wg_hbm, wg_v, sem_w.at[5]),
        pltpu.make_async_copy(wu_hbm, wu_v, sem_w.at[6]),
        pltpu.make_async_copy(wd_hbm, wd_v, sem_w.at[7]),
    ]
    x_copy(0).start()
    for j in range(3):
        wqkv_copy(j).start()
    x_copy(1).start()

    ot[...] = jnp.zeros(ot.shape, F32)
    at_v[:, 0:QG] = jnp.zeros((D, QG), F32)

    def ln1_block(b):
        rows = pl.ds(pl.multiple_of(b * RB, RB), RB)
        xn = _layernorm(x_v[rows, :].astype(F32))
        xn_v[pl.ds(pl.multiple_of(b * (RB // 2), RB // 2), RB // 2), :] = _pack(xn)

    x_copy(0).wait()
    for b in range(2, NRB):
        x_copy(b).start()
    for c in late_copies:
        c.start()
    ln1_block(0)
    for j in range(3):
        wqkv_copy(j).wait()

    def qkv_block(b, carry):
        @pl.when(b + 1 < NRB)
        def _():
            x_copy(b + 1).wait()

        rows = pl.ds(pl.multiple_of(b * RB, RB), RB)
        krows = pl.ds(pl.multiple_of(b * (RB // 2), RB // 2), RB // 2)
        xn = _unpack(xn_v[krows, :])
        q = (jnp.dot(xn, w_v[0], preferred_element_type=F32) * Q_SCALE).astype(BF16)
        qt[:, rows] = pltpu.bitcast(q.T, U32)
        v = jnp.dot(xn, w_v[2], preferred_element_type=F32).astype(BF16)
        vt[:, rows] = v.T.astype(F32)
        k = _pack(jnp.dot(xn, w_v[1], preferred_element_type=F32))
        tiles = [k[:, LANES * j:LANES * (j + 1)] for j in range(D // LANES)]
        rolled = [pltpu.roll(t, 64, 1) for t in tiles]
        lane = lax.broadcasted_iota(I32, (RB // 2, LANES), 1)
        for j in range(NWIN):
            if j % 2 == 0:
                kwin[j, krows, :] = tiles[j // 2]
            else:
                kwin[j, krows, :] = jnp.where(lane < 64, rolled[j // 2], rolled[j // 2 + 1])
        ln1_block(jnp.minimum(b + 1, NRB - 1))
        return carry

    lax.fori_loop(0, NRB, qkv_block, 0)

    def q_operand(h):
        d0 = DH * h
        w = jnp.minimum((d0 >> 6) << 6, D - LANES)
        lo = (d0 - w) >> 1
        q_words = qt[pl.ds(pl.multiple_of(w >> 1, 32), LANES // 2), :]
        rows = lax.broadcasted_iota(I32, q_words.shape, 0)
        q_t = _unpack(jnp.where((rows >= lo) & (rows < lo + DH // 2), q_words, jnp.uint32(0)))
        return q_t, w >> 6

    def v_window(h):
        d0 = DH * h
        u = (d0 >> 3) << 3
        vlo = d0 - u
        return pl.ds(pl.multiple_of(u, 8), VW), vlo, jnp.where(vlo == 0, DH, 0)

    def finish_pv(acc, urows, vlo, one_row, cols):
        arow = lax.broadcasted_iota(I32, acc.shape, 0)
        denom = jnp.sum(jnp.where(arow == one_row, acc, 0.0), axis=0, keepdims=True)
        keep = (arow >= vlo) & (arow < vlo + DH)
        ot[urows, cols] = jnp.where(keep, acc * (1.0 / denom), ot[urows, cols])

    def head_step(h_pv, h_qk):
        if h_qk is not None:
            q_t, widx = q_operand(h_qk)
        if h_pv is not None:
            urows, vlo, one_row = v_window(h_pv)
            v_win = vt[urows, :]
            vrows = lax.broadcasted_iota(I32, v_win.shape, 0)
            v_t = jnp.where(vrows == one_row, 1.0, v_win)

        for g in range(NQG):
            cols = slice(g * QG, (g + 1) * QG)
            acc, mx = None, None
            if h_pv is not None:
                m_old = m_v[0:1, cols]
            for c in range(S // KC):
                keys = slice(c * KC, (c + 1) * KC)
                if h_pv is not None:
                    p = jnp.exp2(s_v[keys, cols] - m_old)
                if h_qk is not None:
                    k_c = _unpack(kwin[widx, c * (KC // 2):(c + 1) * (KC // 2), :])
                    s_new = jnp.dot(k_c, q_t[:, cols], preferred_element_type=F32)
                    s_v[keys, cols] = s_new
                    mc = jnp.max(s_new.reshape(KC // 8, 8, QG), axis=0)
                    mx = mc if mx is None else jnp.maximum(mx, mc)
                if h_pv is not None:
                    o = jnp.dot(v_t[:, keys], p, preferred_element_type=F32)
                    acc = o if acc is None else acc + o
            if h_qk is not None:
                m_v[:, cols] = jnp.broadcast_to(jnp.max(mx, axis=0, keepdims=True), (8, QG))
            if h_pv is not None:
                finish_pv(acc, urows, vlo, one_row, cols)

    late_copies[0].wait()
    late_copies[1].wait()
    wot_v[...] = wo_v[...].T
    head_step(None, 0)

    def head_loop(h, carry):
        head_step(h, h + 1)
        return carry

    lax.fori_loop(0, H - 1, head_loop, 0)

    last_rows, last_vlo, last_one = v_window(H - 1)
    vrows = lax.broadcasted_iota(I32, (VW, S), 0)
    vt[last_rows, :] = jnp.where(vrows == last_one, 1.0, vt[last_rows, :])

    def last_pv_chunks(cols, m_old, acc, chunks):
        for c in chunks:
            keys = slice(c * KC, (c + 1) * KC)
            p = jnp.exp2(s_v[keys, cols] - m_old)
            o = jnp.dot(vt[last_rows, keys], p, preferred_element_type=F32)
            acc = o if acc is None else acc + o
        return acc

    def ln2_block(g, attn_t):
        rows = pl.ds(pl.multiple_of(g * QG, QG), QG)
        h = x_v[rows, :].astype(F32) + attn_t.T
        hn = _layernorm(h)
        o_v[rows, :] = (h + hn).astype(BF16)
        hn = hn.astype(BF16)
        hn_v[pl.ds(pl.multiple_of(g * (QG // 2), QG // 2), QG // 2), :] = pltpu.bitcast(hn, U32)
        return hn

    def route(g, hn):
        rows = pl.ds(pl.multiple_of(g * QG, QG), QG)
        r = lax.dot_general(wr16, hn, (((1,), (1,)), ((), ())), preferred_element_type=F32)
        r_v[:, rows] = r[0:8, :]

    wr16 = jnp.broadcast_to(wr_v[...].reshape(1, D), (16, D))
    cols0 = slice(0, QG)
    finish_pv(last_pv_chunks(cols0, m_v[0:1, cols0], None, range(S // KC)),
              last_rows, last_vlo, last_one, cols0)

    pv_split = [range(0, 3), range(3, 6), range(6, 9), range(9, 12), range(12, 16)]

    def tail_loop(i, carry):
        prev = jnp.maximum(i - 1, 0)
        cols = pl.ds(pl.multiple_of(i * QG, QG), QG)
        ncols = pl.ds(pl.multiple_of(jnp.minimum(i + 1, NQG - 1) * QG, QG), QG)
        hn_prev = ln2_block(prev, at_v[:, pl.ds(pl.multiple_of(prev * QG, QG), QG)])
        o_b = ot[:, cols].astype(BF16)
        m_old = m_v[0:1, ncols]
        acc = None
        for n in range(D // LANES):
            at_v[n * LANES:(n + 1) * LANES, cols] = jnp.dot(
                wot_v[n * LANES:(n + 1) * LANES, :], o_b, preferred_element_type=F32)
            if n == ROUTE_AT:
                route(prev, hn_prev)
            acc = last_pv_chunks(ncols, m_old, acc, pv_split[n])
        finish_pv(acc, last_rows, last_vlo, last_one, ncols)

        @pl.when(i > 0)
        def _():
            out_copy(prev).start()

        return carry

    lax.fori_loop(0, NQG, tail_loop, 0)

    route(NQG - 1, ln2_block(NQG - 1, at_v[:, (NQG - 1) * QG:]))
    out_copy(NQG - 1).start()

    r = r_v[...].astype(BF16).astype(F32)
    r_max = jnp.max(r)
    idx = jnp.min(jnp.where(r == r_max, lax.broadcasted_iota(I32, r.shape, 1), S))
    idx = jnp.minimum(idx, S - 1)
    base = pl.multiple_of((idx >> 4) << 4, 16)
    hit = lax.broadcasted_iota(I32, (16, D), 0) == idx - base
    pair = hn_v[pl.ds(idx >> 1, 1), :]
    word = jnp.where((idx & 1) == 0, pair << 16, pair & jnp.uint32(0xFFFF0000))
    x_sel = jnp.broadcast_to(pltpu.bitcast(word, F32), (16, D)).astype(BF16)

    for c in late_copies[2:]:
        c.wait()
    gate = jnp.dot(x_sel, wg_v[...], preferred_element_type=F32)
    up = jnp.dot(x_sel, wu_v[...], preferred_element_type=F32)
    act = (gate * jax.nn.sigmoid(gate) * up).astype(BF16)
    y = jnp.dot(act, wd_v[...], preferred_element_type=F32)
    y = y * jax.nn.sigmoid(jnp.full((16, D), r_max, F32))
    slab = o_v[pl.ds(base, 16), :].astype(F32)
    fix_v[...] = jnp.where(hit, slab + y, slab).astype(BF16)

    for g in range(NQG):
        out_copy(g).wait()
    fix_copy = pltpu.make_async_copy(fix_v, out_hbm.at[pl.ds(base, 16)], sem_fix)
    fix_copy.start()
    fix_copy.wait()


@jax.jit
def pallas_sequential_preLN__mha_block__moe_arch_mod__prompt_kernel(
    A_x: jax.Array,
    A_wqkv: jax.Array,
    A_wo: jax.Array,
    B_x: jax.Array,
    B_w_r: jax.Array,
    B_w_gate: jax.Array,
    B_w_up: jax.Array,
    B_w_down: jax.Array,
):
    del B_x
    any_spec = pl.BlockSpec(memory_space=pl.ANY)
    out = pl.pallas_call(
        _kernel,
        grid=(),
        in_specs=[any_spec] * 7,
        out_specs=any_spec,
        out_shape=jax.ShapeDtypeStruct((S, D), BF16),
        scratch_shapes=[
            pltpu.VMEM((S, D), BF16),
            pltpu.VMEM((3, D, D), BF16),
            pltpu.VMEM((D, D), BF16),
            pltpu.VMEM((D,), BF16),
            pltpu.VMEM((D, F), BF16),
            pltpu.VMEM((D, F), BF16),
            pltpu.VMEM((F, D), BF16),
            pltpu.VMEM((S // 2, D), U32),
            pltpu.VMEM((NWIN, S // 2, LANES), U32),
            pltpu.VMEM((D // 2, S), U32),
            pltpu.VMEM((D, S), F32),
            pltpu.VMEM((D, S), F32),
            pltpu.VMEM((S, S), F32),
            pltpu.VMEM((8, S), F32),
            pltpu.VMEM((D, D), BF16),
            pltpu.VMEM((D, S), F32),
            pltpu.VMEM((S // 2, D), U32),
            pltpu.VMEM((8, S), F32),
            pltpu.VMEM((S, D), BF16),
            pltpu.VMEM((16, D), BF16),
            pltpu.SemaphoreType.DMA((NRB,)),
            pltpu.SemaphoreType.DMA((8,)),
            pltpu.SemaphoreType.DMA((NQG,)),
            pltpu.SemaphoreType.DMA(()),
        ],
        compiler_params=pltpu.CompilerParams(vmem_limit_bytes=100 * 1024 * 1024),
        name="preln_mha_moe",
    )(A_x.reshape(S, D), A_wqkv, A_wo, B_w_r, B_w_gate, B_w_up, B_w_down)
    return out.reshape(1, S, D)
```

```python
import jax
import jax.numpy as jnp
import numpy as np
from jax import lax
from jax.experimental import pallas as pl
from jax.experimental.pallas import tpu as pltpu

S, D, H, DH, F = 2048, 640, 32, 20, 1536
EPS = 1e-5
LANES = 128

RB = 256
NRB = S // RB
KC = 128
QG = 256
NQG = S // QG
NWIN = 9
VW = 24
Q_SCALE = float(DH ** -0.5 * np.log2(np.e))

BF16, F32, U32, I32 = jnp.bfloat16, jnp.float32, jnp.uint32, jnp.int32


def _layernorm(x):
    mu = jnp.mean(x, axis=-1, keepdims=True)
    xc = x - mu
    var = jnp.mean(xc * xc, axis=-1, keepdims=True)
    return xc * lax.rsqrt(var + EPS)


def _pack(x):
    return pltpu.bitcast(x.astype(BF16), U32)


def _unpack(x):
    return pltpu.bitcast(x, BF16)


def _pv(v_t, p):
    return jnp.dot(v_t, p, preferred_element_type=F32, precision=lax.Precision.DEFAULT)


def _kernel(x_hbm, wqkv_hbm, wo_hbm, wr_hbm, wg_hbm, wu_hbm, wd_hbm, out_hbm,
            x_v, w_v, wo_v, wr_v, wg_v, wu_v, wd_v,
            xn_v, kwin, qt, vt, ot, s_v, m_v, wot_v, at_v, hn_v, r_v, o_v, y_v, fix_v,
            sem_x, sem_w, sem_o, sem_fix):

    def x_copy(b):
        rows = pl.ds(pl.multiple_of(b * RB, RB), RB)
        return pltpu.make_async_copy(x_hbm.at[rows], x_v.at[rows], sem_x.at[b])

    def x01_copy():
        rows = pl.ds(0, 2 * RB)
        return pltpu.make_async_copy(x_hbm.at[rows], x_v.at[rows], sem_x.at[0])

    def out_copy(g):
        rows = pl.ds(pl.multiple_of(g * QG, QG), QG)
        return pltpu.make_async_copy(o_v.at[rows], out_hbm.at[rows], sem_o.at[g])

    def wqkv_copy(j):
        return pltpu.make_async_copy(wqkv_hbm.at[:, pl.ds(j * D, D)], w_v.at[j], sem_w.at[j])

    late_copies = [
        pltpu.make_async_copy(wo_hbm, wo_v, sem_w.at[3]),
        pltpu.make_async_copy(wr_hbm, wr_v, sem_w.at[4]),
        pltpu.make_async_copy(wg_hbm, wg_v, sem_w.at[5]),
        pltpu.make_async_copy(wu_hbm, wu_v, sem_w.at[6]),
        pltpu.make_async_copy(wd_hbm, wd_v, sem_w.at[7]),
    ]

    x01_copy().start()
    wqkv_copy(1).start()

    ot[...] = jnp.zeros(ot.shape, F32)
    at_v[:, 0:QG] = jnp.zeros((D, QG), F32)

    def ln1_block(b):
        for c in range(RB // LANES):
            rows = pl.ds(pl.multiple_of(b * RB + c * LANES, LANES), LANES)
            xn = _layernorm(x_v[rows, :].astype(F32))
            xn_v[pl.ds(pl.multiple_of((b * RB + c * LANES) // 2, LANES // 2), LANES // 2), :] = _pack(xn)

    def project(xn, j):
        return jnp.dot(xn, w_v[j], preferred_element_type=F32)

    def store_q(b, q):
        q = (q * Q_SCALE).astype(BF16)
        qt[:, pl.ds(pl.multiple_of(b * RB, RB), RB)] = pltpu.bitcast(q.T, U32)

    def store_k(b, k):
        krows = pl.ds(pl.multiple_of(b * (RB // 2), RB // 2), RB // 2)
        k = _pack(k)
        tiles = [k[:, LANES * j:LANES * (j + 1)] for j in range(D // LANES)]
        rolled = [pltpu.roll(t, 64, 1) for t in tiles]
        lane = lax.broadcasted_iota(I32, (RB // 2, LANES), 1)
        for j in range(NWIN):
            if j % 2 == 0:
                kwin[j, krows, :] = tiles[j // 2]
            else:
                kwin[j, krows, :] = jnp.where(lane < 64, rolled[j // 2], rolled[j // 2 + 1])

    def store_v(b, v):
        vt[:, pl.ds(pl.multiple_of(b * RB, RB), RB)] = v.astype(BF16).T.astype(F32)

    def qkv_block(b):
        xn = _unpack(xn_v[pl.ds(pl.multiple_of(b * (RB // 2), RB // 2), RB // 2), :])
        store_q(b, project(xn, 0))
        store_v(b, project(xn, 2))
        store_k(b, project(xn, 1))
        ln1_block(jnp.minimum(b + 1, NRB - 1))

    x01_copy().wait()
    wqkv_copy(0).start()
    ln1_block(0)
    xn0 = _unpack(xn_v[0:RB // 2, :])
    wqkv_copy(1).wait()
    wqkv_copy(2).start()
    k0 = project(xn0, 1)
    wqkv_copy(0).wait()
    for b in range(2, NRB):
        x_copy(b).start()
    for c in late_copies:
        c.start()
    q0 = project(xn0, 0)
    store_k(0, k0)
    ln1_block(1)
    wqkv_copy(2).wait()
    x_copy(2).wait()
    v0 = project(xn0, 2)
    store_q(0, q0)
    store_v(0, v0)
    qkv_block(1)

    def qkv_pair(j, carry):
        b = 2 * j
        x_copy(b + 1).wait()

        @pl.when(b + 2 < NRB)
        def _():
            x_copy(b + 2).wait()

        qkv_block(b)
        qkv_block(b + 1)
        return carry

    lax.fori_loop(1, NRB // 2, qkv_pair, 0)

    def q_operand(h):
        d0 = DH * h
        w = jnp.minimum((d0 >> 6) << 6, D - LANES)
        lo = (d0 - w) >> 1
        q_words = qt[pl.ds(pl.multiple_of(w >> 1, 32), LANES // 2), :]
        rows = lax.broadcasted_iota(I32, q_words.shape, 0)
        q_t = _unpack(jnp.where((rows >= lo) & (rows < lo + DH // 2), q_words, jnp.uint32(0)))
        return q_t, w >> 6

    def v_window(h):
        d0 = DH * h
        u = (d0 >> 3) << 3
        vlo = d0 - u
        return pl.ds(pl.multiple_of(u, 8), VW), vlo, jnp.where(vlo == 0, DH, 0)

    def finish_pv(acc, urows, vlo, one_row, cols):
        arow = lax.broadcasted_iota(I32, acc.shape, 0)
        denom = jnp.sum(jnp.where(arow == one_row, acc, 0.0), axis=0, keepdims=True)
        keep = (arow >= vlo) & (arow < vlo + DH)
        ot[urows, cols] = jnp.where(keep, acc * (1.0 / denom), ot[urows, cols])

    def head_step(h_pv, h_qk):
        if h_qk is not None:
            q_t, widx = q_operand(h_qk)
        if h_pv is not None:
            urows, vlo, one_row = v_window(h_pv)
            v_win = vt[urows, :]
            vrows = lax.broadcasted_iota(I32, v_win.shape, 0)
            v_t = jnp.where(vrows == one_row, 1.0, v_win)

        for g in range(NQG):
            cols = slice(g * QG, (g + 1) * QG)
            acc, mx = None, None
            if h_pv is not None:
                m_old = m_v[0:1, cols]
            for c in range(S // KC):
                keys = slice(c * KC, (c + 1) * KC)
                if h_pv is not None:
                    p = jnp.exp2(s_v[keys, cols] - m_old)
                if h_qk is not None:
                    k_c = _unpack(kwin[widx, c * (KC // 2):(c + 1) * (KC // 2), :])
                    s_new = jnp.dot(k_c, q_t[:, cols], preferred_element_type=F32)
                    s_v[keys, cols] = s_new
                    mc = jnp.max(s_new.reshape(KC // 8, 8, QG), axis=0)
                    mx = mc if mx is None else jnp.maximum(mx, mc)
                if h_pv is not None:
                    o = _pv(v_t[:, keys], p)
                    acc = o if acc is None else acc + o
            if h_qk is not None:
                m_v[:, cols] = jnp.broadcast_to(jnp.max(mx, axis=0, keepdims=True), (8, QG))
            if h_pv is not None:
                finish_pv(acc, urows, vlo, one_row, cols)

    late_copies[0].wait()
    late_copies[1].wait()
    wot_v[...] = wo_v[...].T
    head_step(None, 0)

    def head_pair(j, carry):
        h = 2 * j
        head_step(h, h + 1)
        head_step(h + 1, h + 2)
        return carry

    lax.fori_loop(0, (H - 2) // 2, head_pair, 0)
    head_step(H - 2, H - 1)

    last_rows, last_vlo, last_one = v_window(H - 1)
    vrows = lax.broadcasted_iota(I32, (VW, S), 0)
    vt[last_rows, :] = jnp.where(vrows == last_one, 1.0, vt[last_rows, :])

    def last_pv_chunks(cols, m_old, acc, chunks):
        for c in chunks:
            keys = slice(c * KC, (c + 1) * KC)
            p = jnp.exp2(s_v[keys, cols] - m_old)
            o = _pv(vt[last_rows, keys], p)
            acc = o if acc is None else acc + o
        return acc

    def ln2_block(g, attn_t):
        tiles = []
        for t in range(QG // LANES):
            row0 = g * QG + t * LANES
            rows = pl.ds(pl.multiple_of(row0, LANES), LANES)
            h = x_v[rows, :].astype(F32) + attn_t[:, t * LANES:(t + 1) * LANES].T
            hn = _layernorm(h)
            o_v[rows, :] = (h + hn).astype(BF16)
            hn = hn.astype(BF16)
            hn_v[pl.ds(pl.multiple_of(row0 // 2, LANES // 2), LANES // 2), :] = pltpu.bitcast(hn, U32)
            tiles.append(hn)
        return tiles

    def route(g, hn_tiles):
        for t, hn in enumerate(hn_tiles):
            r = lax.dot_general(wr16, hn, (((1,), (1,)), ((), ())), preferred_element_type=F32)
            r_v[:, pl.ds(pl.multiple_of(g * QG + t * LANES, LANES), LANES)] = r[0:8, :]

    wr16 = jnp.broadcast_to(wr_v[...].reshape(1, D), (16, D))
    cols0 = slice(0, QG)
    finish_pv(last_pv_chunks(cols0, m_v[0:1, cols0], None, range(S // KC)),
              last_rows, last_vlo, last_one, cols0)

    pv_split = [range(0, 3), range(3, 6), range(6, 9), range(9, 12), range(12, 16)]

    def tail_step(i, carry):
        prev = jnp.maximum(i - 1, 0)
        cols = pl.ds(pl.multiple_of(i * QG, QG), QG)
        ncols = pl.ds(pl.multiple_of(jnp.minimum(i + 1, NQG - 1) * QG, QG), QG)
        hn_prev = ln2_block(prev, at_v[:, pl.ds(pl.multiple_of(prev * QG, QG), QG)])
        o_b = ot[:, cols].astype(BF16)
        m_old = m_v[0:1, ncols]
        acc = None
        for n in range(D // LANES):
            at_v[n * LANES:(n + 1) * LANES, cols] = jnp.dot(
                wot_v[n * LANES:(n + 1) * LANES, :], o_b, preferred_element_type=F32)
            if n == D // LANES - 1:
                route(prev, hn_prev)
            acc = last_pv_chunks(ncols, m_old, acc, pv_split[n])
        finish_pv(acc, last_rows, last_vlo, last_one, ncols)

        @pl.when(i > 0)
        def _():
            out_copy(prev).start()

        return carry

    lax.fori_loop(0, NQG, tail_step, 0)

    def best_key(r, tok0):
        bits = pltpu.bitcast(r.astype(BF16).astype(F32) + 0.0, I32)
        rank = ((bits ^ ((bits >> 31) & 0x7FFFFFFF)) >> 16) + 32768
        tok = tok0 + lax.broadcasted_iota(I32, r.shape, 1)
        return jnp.max((rank << 11) | (S - 1 - tok))

    def token_of(key):
        return S - 1 - (key & (S - 1))

    def ffn_in(idx):
        pair = hn_v[pl.ds(idx >> 1, 1), :]
        word = jnp.where((idx & 1) == 0, pair << 16, pair & jnp.uint32(0xFFFF0000))
        x_sel = jnp.broadcast_to(pltpu.bitcast(word, F32), (16, D)).astype(BF16)
        gate = jnp.dot(x_sel, wg_v[...], preferred_element_type=F32)
        up = jnp.dot(x_sel, wu_v[...], preferred_element_type=F32)
        return (gate * jax.nn.sigmoid(gate) * up).astype(BF16)

    def ffn_out(act):
        return jnp.dot(act, wd_v[...], preferred_element_type=F32)

    for c in late_copies[2:]:
        c.wait()

    last0 = (NQG - 1) * QG
    key_early = best_key(r_v[:, 0:last0], 0)
    act_early = ffn_in(token_of(key_early))
    route(NQG - 1, ln2_block(NQG - 1, at_v[:, last0:]))
    out_copy(NQG - 1).start()
    y_v[...] = ffn_out(act_early)
    key_last = best_key(r_v[:, last0:], last0)

    idx = token_of(jnp.maximum(key_early, key_last))
    r_sel = jnp.max(r_v[...].astype(BF16).astype(F32))
    gain = jax.nn.sigmoid(jnp.full((16, D), r_sel, F32))
    base = pl.multiple_of((idx >> 4) << 4, 16)
    hit = lax.broadcasted_iota(I32, (16, D), 0) == idx - base
    slab = o_v[pl.ds(base, 16), :].astype(F32)
    for g in range(NQG - 1):
        out_copy(g).wait()

    @pl.when(key_last > key_early)
    def _():
        y_v[...] = ffn_out(ffn_in(token_of(key_last)))

    fix_v[...] = jnp.where(hit, slab + y_v[...] * gain, slab).astype(BF16)
    out_copy(NQG - 1).wait()
    fix_copy = pltpu.make_async_copy(fix_v, out_hbm.at[pl.ds(base, 16)], sem_fix)
    fix_copy.start()
    fix_copy.wait()


@jax.jit
def pallas_sequential_preLN__mha_block__moe_arch_mod__prompt_kernel(
    A_x: jax.Array,
    A_wqkv: jax.Array,
    A_wo: jax.Array,
    B_x: jax.Array,
    B_w_r: jax.Array,
    B_w_gate: jax.Array,
    B_w_up: jax.Array,
    B_w_down: jax.Array,
):
    del B_x
    any_spec = pl.BlockSpec(memory_space=pl.ANY)
    out = pl.pallas_call(
        _kernel,
        grid=(),
        in_specs=[any_spec] * 7,
        out_specs=any_spec,
        out_shape=jax.ShapeDtypeStruct((S, D), BF16),
        scratch_shapes=[
            pltpu.VMEM((S, D), BF16),
            pltpu.VMEM((3, D, D), BF16),
            pltpu.VMEM((D, D), BF16),
            pltpu.VMEM((D,), BF16),
            pltpu.VMEM((D, F), BF16),
            pltpu.VMEM((D, F), BF16),
            pltpu.VMEM((F, D), BF16),
            pltpu.VMEM((S // 2, D), U32),
            pltpu.VMEM((NWIN, S // 2, LANES), U32),
            pltpu.VMEM((D // 2, S), U32),
            pltpu.VMEM((D, S), F32),
            pltpu.VMEM((D, S), F32),
            pltpu.VMEM((S, S), F32),
            pltpu.VMEM((8, S), F32),
            pltpu.VMEM((D, D), BF16),
            pltpu.VMEM((D, S), F32),
            pltpu.VMEM((S // 2, D), U32),
            pltpu.VMEM((8, S), F32),
            pltpu.VMEM((S, D), BF16),
            pltpu.VMEM((16, D), F32),
            pltpu.VMEM((16, D), BF16),
            pltpu.SemaphoreType.DMA((NRB,)),
            pltpu.SemaphoreType.DMA((8,)),
            pltpu.SemaphoreType.DMA((NQG,)),
            pltpu.SemaphoreType.DMA(()),
        ],
        compiler_params=pltpu.CompilerParams(vmem_limit_bytes=100 * 1024 * 1024),
        name="preln_mha_moe",
    )(A_x.reshape(S, D), A_wqkv, A_wo, B_w_r, B_w_gate, B_w_up, B_w_down)
    return out.reshape(1, S, D)
```
